```python
import jax
import jax.numpy as jnp

def _softmax(x, axis=-1):
    return jax.nn.softmax(x, axis=axis)
def _gelu(x):
    return jax.nn.gelu(x, approximate=True)
def _silu(x):
    return jax.nn.silu(x)
def _sigmoid(x):
    return jax.nn.sigmoid(x)
def _layernorm(x, axis=-1, eps=1e-5):
    m = jnp.mean(x, axis=axis, keepdims=True)
    v = jnp.var(x, axis=axis, keepdims=True)
    return (x - m) / jnp.sqrt(v + eps)
def _scatter_add(tgt, idx, src, axis=0):
    return tgt.at[idx].add(src)
def _segment_sum(src, seg, n):
    return jax.ops.segment_sum(src, seg, n)
class _Rng:
    def __init__(self, key):
        self._k = key
    def _next(self):
        self._k, sub = jax.random.split(self._k)
        return sub
    def normal(self, shape):
        return jax.random.normal(self._next(), shape, dtype=jnp.bfloat16)
    def randint(self, lo, hi, shape):
        return jax.random.randint(self._next(), shape, lo, hi, dtype=jnp.int32)
    def uniform(self, shape, lo=0.0, hi=1.0):
        return jax.random.uniform(self._next(), shape, jnp.bfloat16, lo, hi)
    def permutation(self, n):
        return jax.random.permutation(self._next(), n)


kernel_name = 'gated_mix__mha_block_cached__moe_arch_mod__decode'

def setup_inputs():
    _rng = _Rng(jax.random.key(int.from_bytes(__import__("os").urandom(4), "little")))
    _w = (lambda a: (lambda t: t.astype(jnp.bfloat16) if jnp.issubdtype(t.dtype, jnp.floating) else t)(jnp.asarray(a)))
    def _A_setup():
        B, Sq, D = 4, 1, 1024
        H, Sk, Dh = 32, 8192, 128
        return {
            "x": _w((lambda *s: _rng.normal(s) * 0.05)(B, Sq, D)),
            "k_cache": _w((lambda *s: _rng.normal(s) * 0.05)(B, H, Sk, Dh)),
            "v_cache": _w((lambda *s: _rng.normal(s) * 0.05)(B, H, Sk, Dh)),
            "wq": _w((lambda *s: _rng.normal(s) * 0.05)(D, H * Dh) * (D ** -0.5)),
            "wo": _w((lambda *s: _rng.normal(s) * 0.05)(H * Dh, D) * ((H * Dh) ** -0.5)),
        }
    _A_in = _A_setup()

    def _B_setup():
        B, S, D, F, C = 4, 1, 1024, 3584, 1
        return {
            "x": _w((lambda *s: _rng.normal(s) * 0.05)(B, S, D)),
            "w_r": _w((lambda *s: _rng.normal(s) * 0.05)(D)),
            "w_gate": _w((lambda *s: _rng.normal(s) * 0.05)(D, F)),
            "w_up": _w((lambda *s: _rng.normal(s) * 0.05)(D, F)),
            "w_down": _w((lambda *s: _rng.normal(s) * 0.05)(F, D)),
        }
    _B_in = _B_setup()

    return {
        "A_x": _A_in["x"],
        "A_k_cache": _A_in["k_cache"],
        "A_v_cache": _A_in["v_cache"],
        "A_wq": _A_in["wq"],
        "A_wo": _A_in["wo"],
        "B_x": _B_in["x"],
        "B_w_r": _B_in["w_r"],
        "B_w_gate": _B_in["w_gate"],
        "B_w_up": _B_in["w_up"],
        "B_w_down": _B_in["w_down"],
        "gate_w": _w((lambda *s: _rng.normal(s) * 0.05)(1024)),
    }

def reference(A_x, A_k_cache, A_v_cache, A_wq, A_wo, B_x, B_w_r, B_w_gate, B_w_up, B_w_down, gate_w):
    def _A_ref(x, k_cache, v_cache, wq, wo):
        B, Sq, D = x.shape
        H, Dh = 32, 128
        q = (lambda x, *d: x.transpose(*d))((x @ wq).reshape(B, Sq, H, Dh), 0, 2, 1, 3)
        scores = jnp.einsum("bhqd,bhkd->bhqk", q, k_cache) * (Dh ** -0.5)
        p = _softmax(scores, axis=-1)
        o = jnp.einsum("bhqk,bhkd->bhqd", p, v_cache)
        return (lambda x, *d: x.transpose(*d))(o, 0, 2, 1, 3).reshape(B, Sq, H * Dh) @ wo

    def _B_ref(x, w_r, w_gate, w_up, w_down):
        B, S, D = x.shape
        C = 1
        r = x @ w_r
        idx = jnp.argsort(-r, axis=-1)[:, :C]
        idx_e = jnp.repeat(idx.reshape(B, C, 1), D, axis=2)
        x_sel = jnp.take_along_axis(x, idx_e, axis=1)
        g = _silu(x_sel @ w_gate)
        u = x_sel @ w_up
        y = (g * u) @ w_down
        r_sel = _sigmoid(jnp.take_along_axis(r, idx, axis=1))
        y = y * r_sel.reshape(B, C, 1)
        b_off = (jnp.arange(B) * S).reshape(B, 1)
        flat_idx = (idx + b_off).reshape(B * C)
        zero = (x * 0.0).reshape(B * S, D)
        upd = _scatter_add(zero, flat_idx, y.reshape(B * C, D), axis=0)
        return x + upd.reshape(B, S, D)

    x = A_x
    g = _sigmoid((x * gate_w).sum(-1, keepdims=True))
    a = _A_ref(x, A_k_cache, A_v_cache, A_wq, A_wo)
    b = _B_ref(x, B_w_r, B_w_gate, B_w_up, B_w_down)
    return g * a + (1 - g) * b
```

```python
import functools

import jax
import jax.experimental.pallas as pl
import jax.experimental.pallas.tpu as pltpu
import jax.numpy as jnp

B, D, H, SK, DH, F = 4, 1024, 32, 8192, 128, 3584

M = 8
BLK = 256
LEAD = 192
CUT = BLK - LEAD
NB = 16
G = NB // B
CH = G * BLK
NC = SK // CH
NS = 2 * NC
SLOTS = 2 * NS
AHEAD = 3
BAND = 8 * D // 128

NW_FFN = D * F // (128 * NB * BLK)
NW_ATT = D * H * DH // (128 * NB * BLK)
T_WU = NW_FFN
T_WD = T_WU + NW_FFN
T_WO = T_WD + NW_FFN - 1
T_END = T_WO + NW_ATT
T_ACT = (T_WO + 1) * NS
assert T_END < H - 1 and T_ACT + F // 128 + NB < (H - 1) * NS and AHEAD < NC

F32, BF16 = jnp.float32, jnp.bfloat16


def _plan(heavy_rows, light_rows):
    order = list(range(0, NB, 2)) + list(range(1, NB, 2))
    light = order[NB // 2 - 1::NB // 2]
    heavy = [s for s in order if s not in light]
    copies = []
    for queue, blocks, rows, phase in ((1, heavy, heavy_rows, 0.0), (0, light, light_rows, 0.5)):
        n = len(blocks) * BLK // rows
        copies += [((i + phase) / n, (blocks[i * rows // BLK], i * rows % BLK, rows, queue))
                   for i in range(n)]
    return [copy for _, copy in sorted(copies)]


def _split_at_cut(plan, blocks):
    out = []
    for s, row, rows, queue in plan:
        if s in blocks and row < CUT < row + rows:
            out += [(s, row, CUT - row, queue), (s, CUT, row + rows - CUT, queue)]
        else:
            out.append((s, row, rows, queue))
    return out


KV_PLAN = _split_at_cut(_plan(128, 32), range(G - 1, NB, G))
W_PLAN = _split_at_cut(_plan(128, 32), [NB - 1])
WQ_PLAN = _split_at_cut(_plan(64, 16), [NB - 1])
LAST_PLAN = _split_at_cut(_plan(32, 16), [NB - 1])


def _last_band(s, row):
    return ((s + 1) * NW_FFN * BLK - CUT + row) // BAND % (F // 8)


def _last_stages(sizes):
    done = {_last_band(s, row): i for i, (s, row, _, _) in enumerate(LAST_PLAN)}
    bands = sorted(done, key=done.get)
    stages = []
    for size in sizes:
        stages.append(sorted(bands[:size]))
        bands = bands[size:]
    assert not bands
    return stages


LAST_STAGES = _last_stages((48, 16))


def _kernel(x_hbm, k_hbm, v_hbm, wq_hbm, wo_hbm, wr_hbm, wg_hbm, wu_hbm, wd_hbm, gw_hbm,
            out_ref,
            ring, wq, wo, wg, wu, wd, x_in, wr, gw,
            xs, qs, run_max, run_sum, run_pv, heads, scores, acts, last_acts, y_acc, a_acc, mix,
            ring_sem, w_sem, last_sem, small_sem):

    def wait_all(buf, sem):
        pltpu.make_async_copy(buf, buf, sem).wait()

    def start_weights(src, dst, sem, c, plan=W_PLAN):
        stride = dst.shape[0] // NB
        last = c == stride * 8 // BLK - 1
        for s, row, rows, queue in plan:
            tile = s * stride + (LEAD + row) // 8 + c * (BLK // 8)
            if s == NB - 1 and row >= CUT:
                tile = jnp.where(last, (row - CUT) // 8, tile)
            at = pl.ds(tile, rows // 8)
            pltpu.make_async_copy(src.at[at], dst.at[at], sem).start(priority=queue)

    def start_last(copies):
        stage = {band: i for i, bands in enumerate(LAST_STAGES) for band in bands}
        for s, row, rows, queue in copies:
            band = _last_band(s, row)
            at = pl.ds((band * BAND + (LEAD + row) % BAND) // 8, rows // 8)
            pltpu.make_async_copy(
                wd_hbm.at[at], wd.at[at], last_sem.at[stage[band]]).start(priority=queue)

    def start_kv(src, h, c, slot):
        last = c == NC - 1
        next_slot = jnp.where(last, (slot + NS) % SLOTS, slot)
        in_range = jnp.logical_or(h < H - 1, jnp.logical_not(last))

        def start(s, row, rows, queue, slot):
            b, g = divmod(s, G)
            first = b * H * SK + g * (SK // G) + LEAD + row + (h * SK + c * BLK)
            pltpu.make_async_copy(src.at[pl.ds(pl.multiple_of(first, 16), rows)],
                                  ring.at[slot, b, pl.ds(g * BLK + row, rows)],
                                  ring_sem.at[slot]).start(priority=queue)

        for s, row, rows, queue in KV_PLAN:
            if s % G == G - 1 and row >= CUT:
                pl.when(in_range)(functools.partial(start, s, row, rows, queue, next_slot))
            else:
                start(s, row, rows, queue, slot)

    def fold(a, op):
        return functools.reduce(op, [a[:, i:i + 128] for i in range(0, CH, 128)])

    def per_batch(fn):
        parts = [fn(b) for b in range(B)]
        row = jax.lax.broadcasted_iota(jnp.int32, parts[0].shape, 0)
        merged = jnp.zeros_like(parts[0])
        for b in range(B):
            merged = jnp.where(row == b, parts[b], merged)
        return merged

    def columns(w, c):
        per_band = w.shape[0] // (D // 8)
        return jnp.concatenate([w[c + i * per_band] for i in range(D // 8)], axis=0)

    def bands_of(w, bands):
        return jnp.concatenate(
            [jnp.concatenate([w[r * (D // 128) + c] for r in bands], axis=0)
             for c in range(D // 128)], axis=1)

    def project(h):
        a_acc[...] += jnp.dot(heads[h], bands_of(wo, [h * (DH // 8) + i for i in range(DH // 8)]),
                              preferred_element_type=F32)

    @pl.loop(0, NW_ATT)
    def _(c):
        start_weights(wq_hbm, wq, w_sem.at[0], c, WQ_PLAN)

    small = ((x_hbm, x_in), (wr_hbm, wr), (gw_hbm, gw))
    for i, (src, dst) in enumerate(small):
        pltpu.make_async_copy(src, dst, small_sem.at[i]).start()
    for src, slot in ((k_hbm, NC - 1), (v_hbm, NS - 1)):
        for b in range(B):
            pltpu.make_async_copy(src.at[pl.ds(b * H * SK, LEAD)],
                                  ring.at[slot, b, pl.ds(CH - LEAD, LEAD)],
                                  ring_sem.at[slot]).start(priority=b % 2)

    def consume(t):
        h, r, slot = t // NS, t % NS, t % SLOTS

        @pl.when(t == 0)
        def _():
            for i, (src, dst) in enumerate(small):
                pltpu.make_async_copy(src, dst, small_sem.at[i]).wait()
            xs[...] = jnp.zeros(xs.shape, F32)
            xs[0:B, :] = x_in[...].astype(F32)
            y_acc[...] = jnp.zeros(y_acc.shape, F32)
            a_acc[...] = jnp.zeros(a_acc.shape, F32)
            wait_all(wq, w_sem.at[0])

        @pl.when(r == 0)
        def _():
            qs[...] = jnp.dot(xs[...].astype(BF16), columns(wq, h),
                              preferred_element_type=F32).astype(BF16)
            run_max[...] = jnp.full(run_max.shape, -jnp.inf, F32)
            run_sum[...] = jnp.zeros(run_sum.shape, F32)
            run_pv[...] = jnp.zeros(run_pv.shape, F32)

        @pl.when(r < NC)
        def _():
            wait_all(ring.at[slot], ring_sem.at[slot])
            q = qs[...]
            s = per_batch(lambda b: jax.lax.dot_general(
                q, ring[slot, b], (((1,), (1,)), ((), ())),
                preferred_element_type=F32)) * (DH ** -0.5)
            scores[r] = s
            run_max[...] = jnp.maximum(run_max[...], fold(s, jnp.maximum))

        @pl.when(r >= NC)
        def _():
            p = jnp.exp(scores[r - NC] - jnp.max(run_max[...], axis=-1, keepdims=True))
            run_sum[...] += fold(p, jnp.add)
            p16 = p.astype(BF16)
            wait_all(ring.at[slot], ring_sem.at[slot])
            run_pv[...] += per_batch(
                lambda b: jnp.dot(p16, ring[slot, b], preferred_element_type=F32))

    def request(t):
        h, r, slot = t // NS, t % NS, t % SLOTS

        @pl.when(jnp.logical_and(h < H, r < NC))
        def _():
            start_kv(k_hbm, h, r, slot)

        @pl.when(r >= NC)
        def _():
            start_kv(v_hbm, h, r - NC, slot)

        n = len(LAST_PLAN)
        for i in range(AHEAD):
            pl.when(t == H * NS + i)(functools.partial(
                start_last, LAST_PLAN[i * n // AHEAD:(i + 1) * n // AHEAD]))

    def side_jobs(t):
        h, r = t // NS, t % NS

        for lo, hi, src, dst, i in ((0, T_WU, wg_hbm, wg, 1), (T_WU, T_WD, wu_hbm, wu, 2),
                                    (T_WD, T_WO, wd_hbm, wd, 3), (T_WO, T_END, wo_hbm, wo, 4)):
            pl.when(jnp.logical_and(r == 2, jnp.logical_and(h >= lo, h < hi)))(
                functools.partial(start_weights, src, dst, w_sem.at[i], h - lo))

        @pl.when(h == 1)
        def _():
            for row in range(0, BLK, BAND):
                band = _last_band(0, row) + r * (NW_FFN * BLK // BAND)
                band = jnp.where(band >= F // 8, band - F // 8, band)
                wd[pl.ds(band * (D // 128), D // 128)] = jnp.zeros((D // 128, 8, 128), BF16)

        @pl.when(r == NS - 1)
        def _():
            denom = jnp.sum(run_sum[...], axis=-1, keepdims=True)
            heads[h] = (run_pv[...] / denom).astype(BF16)

        @pl.when(t == T_ACT - 1)
        def _():
            wait_all(wg, w_sem.at[1])
            wait_all(wu, w_sem.at[2])
            wait_all(wd.at[pl.ds(0, (NW_FFN - 1) * NB * BLK // 8)], w_sem.at[3])

        @pl.when(jnp.logical_and(t >= T_ACT, t < T_ACT + F // 128))
        def _():
            c = t - T_ACT
            x16 = xs[...].astype(BF16)
            g = jnp.dot(x16, columns(wg, c), preferred_element_type=F32)
            u = jnp.dot(x16, columns(wu, c), preferred_element_type=F32)
            act = (g * jax.nn.sigmoid(g)) * u
            acts[c] = act
            y_acc[...] += jnp.dot(act.astype(BF16), bands_of(wd, [c * 16 + i for i in range(16)]),
                                  preferred_element_type=F32)

        for i, bands in enumerate(LAST_STAGES):
            @pl.when(t == T_ACT + F // 128 + i)
            def _():
                runs = []
                for band in bands:
                    if runs and runs[-1][1] == band and band % 16:
                        runs[-1][1] += 1
                    else:
                        runs.append([band, band + 1])
                last_acts[i][...] = jnp.concatenate(
                    [acts[lo // 16, :, pl.ds(lo % 16 * 8, (hi - lo) * 8)] for lo, hi in runs],
                    axis=1).astype(BF16)

        @pl.when(t == (H - 1) * NS)
        def _():
            x = xs[...]
            router = jax.nn.sigmoid(
                jnp.sum(x * wr[...].astype(F32).reshape(1, D), axis=-1, keepdims=True))
            gate = jax.nn.sigmoid(
                jnp.sum(x * gw[...].astype(F32).reshape(1, D), axis=-1, keepdims=True))
            y_acc[...] = (1.0 - gate) * (x + (x * 0.0 + y_acc[...] * router))
            mix[0] = jnp.broadcast_to(gate, (M, 128))
            mix[1] = jnp.broadcast_to((1.0 - gate) * router, (M, 128))
            wait_all(wo, w_sem.at[4])

        @pl.when(h == H - 1)
        def _():
            last = r == NS - 1
            lo = jnp.where(last, H - 1, jnp.minimum(r * 3, H - 1))
            hi = jnp.where(last, H, jnp.minimum((r + 1) * 3, H - 1))
            pl.loop(lo, hi)(project)

    @pl.loop(-AHEAD, H * NS)
    def _(t):
        pl.when(t >= 0)(functools.partial(consume, t))
        request(t + AHEAD)
        pl.when(t >= 0)(functools.partial(side_jobs, t))

    def wide(a):
        return jnp.concatenate([a] * (D // 128), axis=1)

    out = wide(mix[0]) * a_acc[...] + y_acc[...]
    for i, bands in enumerate(LAST_STAGES):
        wait_all(wd.at[pl.ds(0, len(bands) * (D // 128))], last_sem.at[i])
        out += wide(mix[1]) * jnp.dot(last_acts[i][...], bands_of(wd, bands),
                                      preferred_element_type=F32)
    out_ref[...] = out[0:B, :].astype(out_ref.dtype)


def _tiles(w):
    rows, cols = w.shape
    return w.reshape(rows // 8, 8, cols // 128, 128).transpose(0, 2, 1, 3).reshape(-1, 8, 128)


@jax.jit
def pallas_gated_mix__mha_block_cached__moe_arch_mod__decode_kernel(
    A_x: jax.Array,
    A_k_cache: jax.Array,
    A_v_cache: jax.Array,
    A_wq: jax.Array,
    A_wo: jax.Array,
    B_x: jax.Array,
    B_w_r: jax.Array,
    B_w_gate: jax.Array,
    B_w_up: jax.Array,
    B_w_down: jax.Array,
    gate_w: jax.Array,
):
    del B_x
    dma_sem = pltpu.SemaphoreType.DMA
    out = pl.pallas_call(
        _kernel,
        out_shape=jax.ShapeDtypeStruct((B, D), BF16),
        in_specs=[pl.BlockSpec(memory_space=pl.ANY)] * 10,
        out_specs=pl.BlockSpec(memory_space=pltpu.VMEM),
        scratch_shapes=[
            pltpu.VMEM((SLOTS, B, CH, DH), BF16),
            pltpu.VMEM((D * H * DH // 1024, 8, 128), BF16),
            pltpu.VMEM((D * H * DH // 1024, 8, 128), BF16),
            pltpu.VMEM((D * F // 1024, 8, 128), BF16),
            pltpu.VMEM((D * F // 1024, 8, 128), BF16),
            pltpu.VMEM((D * F // 1024, 8, 128), BF16),
            pltpu.VMEM((B, D), BF16),
            pltpu.VMEM((D,), BF16),
            pltpu.VMEM((D,), BF16),
            pltpu.VMEM((M, D), F32),
            pltpu.VMEM((M, DH), BF16),
            pltpu.VMEM((M, 128), F32),
            pltpu.VMEM((M, 128), F32),
            pltpu.VMEM((M, DH), F32),
            pltpu.VMEM((H, M, DH), BF16),
            pltpu.VMEM((NC, M, CH), F32),
            pltpu.VMEM((F // 128, M, 128), F32),
            [pltpu.VMEM((M, 8 * len(bands)), BF16) for bands in LAST_STAGES],
            pltpu.VMEM((M, D), F32),
            pltpu.VMEM((M, D), F32),
            pltpu.VMEM((2, M, 128), F32),
            dma_sem((SLOTS,)),
            dma_sem((5,)),
            dma_sem((len(LAST_STAGES),)),
            dma_sem((3,)),
        ],
        compiler_params=pltpu.CompilerParams(
            vmem_limit_bytes=96 * 1024 * 1024,
            disable_bounds_checks=True,
            disable_semaphore_checks=True),
    )(A_x.reshape(B, D), A_k_cache.reshape(-1, DH), A_v_cache.reshape(-1, DH),
      _tiles(A_wq), _tiles(A_wo), B_w_r, _tiles(B_w_gate), _tiles(B_w_up), _tiles(B_w_down),
      gate_w)
    return out.reshape(B, 1, D)
```

```python
import functools

import jax
import jax.experimental.pallas as pl
import jax.experimental.pallas.tpu as pltpu
import jax.numpy as jnp

B, D, H, SK, DH, F = 4, 1024, 32, 8192, 128, 3584

M = 8
BLK = 256
LEAD = 192
CUT = BLK - LEAD
NB = 8
G = 4
CH = G * BLK
NC = SK // CH
NS = 2 * NC
SLOTS = 2 * NS
AHEAD = 3
WD_AHEAD = 4

NR_FFN = D * F // (128 * NB * BLK)
NR_ATT = D * H * DH // (128 * NB * BLK)
EVERY = 8
T_ACT = (2 * NR_FFN + 1) * EVERY
T_OUT = (H - 1) * NS
assert (2 * NR_FFN + NR_ATT) * EVERY < T_OUT and T_ACT + F // 128 < T_OUT and AHEAD < NC

F32, BF16 = jnp.float32, jnp.bfloat16


def _plan(heavy, light):
    copies = []
    for queue, blocks, sizes, phase in ((1, range(NB - 1), heavy, 0.0), (0, [NB - 1], light, 0.5)):
        for i, s in enumerate(blocks):
            row = 0
            for rows in sizes:
                assert not row < CUT < row + rows
                copies.append(((i * BLK + row + phase * rows) / len(blocks), (s, row, rows, queue)))
                row += rows
            assert row == BLK
    return [copy for _, copy in sorted(copies)]


PLAN = _plan((CUT, LEAD), (32,) * 8)
FIRST_PLAN = _plan((32,) * 8, (16,) * 16)


def _kernel(x_hbm, k_hbm, v_hbm, wq_hbm, wo_hbm, wr_hbm, wg_hbm, wu_hbm, wd_hbm, gw_hbm,
            out_ref,
            ring, wq, wo, wg, wu, wd, x_in, wr, gw,
            xs, mix, qs, run_max, run_sum, run_pv, heads, scores, acts, a_acc,
            ring_sem, w_sem, wd_sem, small_sem):

    def wait_all(buf, sem):
        pltpu.make_async_copy(buf, buf, sem).wait()

    def block_tile(w, c, s):
        stride = w.shape[0] // NB
        return s * stride + LEAD // 8 + ((c & 1) * (stride // 2) + (c >> 1) * (BLK // 8))

    def wrap(w, tile):
        return jnp.where(tile >= w.shape[0], tile - w.shape[0], tile)

    def start_round(src, dst, sem_of, c, plan=PLAN):
        for s, row, rows, queue in plan:
            tile = block_tile(dst, c, s) + row // 8
            if s == NB - 1 and row >= CUT:
                tile = wrap(dst, tile)
            at = pl.ds(tile, rows // 8)
            pltpu.make_async_copy(src.at[at], dst.at[at], sem_of(s)).start(priority=queue)

    def start_wd(c):
        start_round(wd_hbm, wd, lambda s: wd_sem.at[c * NB + s], c)

    def start_kv(src, h, c, slot):
        last = c == NC - 1
        next_slot = jnp.where(last, (slot + NS) % SLOTS, slot)
        in_range = jnp.logical_or(h < H - 1, jnp.logical_not(last))

        @pl.loop(0, B, step=NB // G)
        def _(b0):
            def start(s, row, rows, queue, slot):
                b, g = divmod(s, G)
                first = b * H * SK + g * (SK // G) + LEAD + row + ((b0 * H + h) * SK + c * BLK)
                pltpu.make_async_copy(src.at[pl.ds(pl.multiple_of(first, 16), rows)],
                                      ring.at[slot, b0 + b, pl.ds(g * BLK + row, rows)],
                                      ring_sem.at[slot]).start(priority=queue)

            for s, row, rows, queue in PLAN:
                if s % G == G - 1 and row >= CUT:
                    pl.when(in_range)(functools.partial(start, s, row, rows, queue, next_slot))
                else:
                    start(s, row, rows, queue, slot)

    def fold(a, op):
        return functools.reduce(op, [a[:, i:i + 128] for i in range(0, CH, 128)])

    def wide(a):
        return jnp.concatenate([a] * (D // 128), axis=1)

    def per_batch(fn):
        parts = [fn(b) for b in range(B)]
        row = jax.lax.broadcasted_iota(jnp.int32, parts[0].shape, 0)
        merged = jnp.zeros_like(parts[0])
        for b in range(B):
            merged = jnp.where(row == b, parts[b], merged)
        return merged

    def x_times(w, c):
        per_band = w.shape[0] // (D // 8)
        cols = jnp.concatenate([w[c + i * per_band] for i in range(D // 8)], axis=0)
        return jnp.dot(xs[...].astype(BF16), cols, preferred_element_type=F32)

    def project(h):
        n = D // 128
        rows = jnp.concatenate(
            [jnp.concatenate([wo[(h * (DH // 8) + i) * n + c] for i in range(DH // 8)], axis=0)
             for c in range(n)], axis=1)
        a_acc[...] += jnp.dot(heads[h], rows, preferred_element_type=F32)

    start_round(wq_hbm, wq, lambda s: w_sem.at[0], 0, FIRST_PLAN)
    pl.loop(1, NR_ATT)(functools.partial(start_round, wq_hbm, wq, lambda s: w_sem.at[0]))

    small = ((x_hbm, x_in), (wr_hbm, wr), (gw_hbm, gw))
    for i, (src, dst) in enumerate(small):
        pltpu.make_async_copy(src, dst, small_sem.at[i]).start()
    for src, slot in ((k_hbm, NC - 1), (v_hbm, NS - 1)):
        for b in range(B):
            pltpu.make_async_copy(src.at[pl.ds(b * H * SK, LEAD)],
                                  ring.at[slot, b, pl.ds(CH - LEAD, LEAD)],
                                  ring_sem.at[slot]).start(priority=b % 2)

    def consume(t):
        h, r, slot = t // NS, t % NS, t % SLOTS

        @pl.when(t == 0)
        def _():
            for i, (src, dst) in enumerate(small):
                pltpu.make_async_copy(src, dst, small_sem.at[i]).wait()
            xs[...] = jnp.zeros(xs.shape, F32)
            xs[0:B, :] = x_in[...].astype(F32)
            a_acc[...] = jnp.zeros(a_acc.shape, F32)
            wait_all(wq, w_sem.at[0])

        @pl.when(r == 0)
        def _():
            qs[...] = x_times(wq, h).astype(BF16)
            run_max[...] = jnp.full(run_max.shape, -jnp.inf, F32)
            run_sum[...] = jnp.zeros(run_sum.shape, F32)
            run_pv[...] = jnp.zeros(run_pv.shape, F32)

        @pl.when(r < NC)
        def _():
            wait_all(ring.at[slot], ring_sem.at[slot])
            q = qs[...]
            s = per_batch(lambda b: jax.lax.dot_general(
                q, ring[slot, b], (((1,), (1,)), ((), ())),
                preferred_element_type=F32)) * (DH ** -0.5)
            scores[r] = s
            run_max[...] = jnp.maximum(run_max[...], fold(s, jnp.maximum))

        @pl.when(r >= NC)
        def _():
            p = jnp.exp(scores[r - NC] - jnp.max(run_max[...], axis=-1, keepdims=True))
            run_sum[...] += fold(p, jnp.add)
            p16 = p.astype(BF16)
            wait_all(ring.at[slot], ring_sem.at[slot])
            run_pv[...] += per_batch(
                lambda b: jnp.dot(p16, ring[slot, b], preferred_element_type=F32))

    def request(t):
        h, r, slot = t // NS, t % NS, t % SLOTS
        pl.when(jnp.logical_and(h < H, r < NC))(functools.partial(start_kv, k_hbm, h, r, slot))
        pl.when(r >= NC)(functools.partial(start_kv, v_hbm, h, r - NC, slot))

        @pl.when(h == H)
        def _():
            pl.loop(jnp.minimum(2 * r, WD_AHEAD), jnp.minimum(2 * r + 2, WD_AHEAD))(start_wd)

    def side_jobs(t):
        h, r = t // NS, t % NS

        @pl.when(t % EVERY == 2)
        def _():
            c = t // EVERY
            for i, (src, dst, rounds) in enumerate(
                    ((wg_hbm, wg, NR_FFN), (wu_hbm, wu, NR_FFN), (wo_hbm, wo, NR_ATT)), 1):
                pl.when(jnp.logical_and(c >= 0, c < rounds))(
                    functools.partial(start_round, src, dst, lambda s: w_sem.at[i], c))
                c = c - rounds

        @pl.when(r == NS - 1)
        def _():
            denom = jnp.sum(run_sum[...], axis=-1, keepdims=True)
            heads[h] = (run_pv[...] / denom).astype(BF16)

        @pl.when(t == T_ACT - 1)
        def _():
            gate, router = [
                jax.nn.sigmoid(jnp.sum(xs[...] * w[...].astype(F32).reshape(1, D),
                                       axis=-1, keepdims=True)) for w in (gw, wr)]
            mix[0] = jnp.broadcast_to(gate, (M, 128))
            mix[1] = jnp.broadcast_to((1.0 - gate) * router, (M, 128))
            wait_all(wg, w_sem.at[1])
            wait_all(wu, w_sem.at[2])

        @pl.when(jnp.logical_and(t >= T_ACT, t < T_ACT + F // 128))
        def _():
            c = t - T_ACT
            g = x_times(wg, c)
            act = (g * jax.nn.sigmoid(g)) * x_times(wu, c) * mix[1]
            for b in range(B):
                acts[b, pl.ds(pl.multiple_of(c * 128, 128), 128), :] = (
                    jnp.broadcast_to(act[b:b + 1, :], (128, 128)).T)

        @pl.when(t == T_OUT)
        def _():
            wait_all(wo, w_sem.at[3])

        @pl.when(t >= T_OUT)
        def _():
            last = r == NS - 1
            lo = jnp.where(last, H - 1, jnp.minimum(r * 3, H - 1))
            hi = jnp.where(last, H, jnp.minimum((r + 1) * 3, H - 1))
            pl.loop(lo, hi)(project)

    @pl.loop(-AHEAD, H * NS)
    def _(t):
        pl.when(t >= 0)(functools.partial(consume, t))
        request(t + AHEAD)
        pl.when(t >= 0)(functools.partial(side_jobs, t))

    x, gate = xs[...], wide(mix[0])
    a_acc[...] = gate * a_acc[...] + (1.0 - gate) * (x + x * 0.0)

    def down(c, sums):
        pl.when(c + WD_AHEAD < NR_FFN)(functools.partial(start_wd, c + WD_AHEAD))
        for s in (NB - 1, *range(NB - 1)):
            wait_all(wd.at[pl.ds(0, BLK // 8)], wd_sem.at[c * NB + s])
            for j in range(0, BLK // 8, D // 128):
                tile = block_tile(wd, c, s) + j
                tile = pl.multiple_of(wrap(wd, tile) if s == NB - 1 else tile, 8)
                w = jnp.concatenate([wd[tile + k].astype(F32) for k in range(D // 128)], axis=1)
                sums = [sums[b] + wide(acts[b, pl.ds(tile, 8), :]) * w for b in range(B)]
        return sums

    sums = jax.lax.fori_loop(0, NR_FFN, down, [jnp.zeros((8, D), F32)] * B)

    def merge(u, v, k):
        low = (jax.lax.broadcasted_iota(jnp.int32, u.shape, 0) & k) == 0
        return jnp.where(low, u, v) + pltpu.roll(jnp.where(low, v, u), 8 - k, 0)

    y = merge(merge(sums[0], sums[1], 1), merge(sums[2], sums[3], 1), 2)
    out = a_acc[...] + y + pltpu.roll(y, 4, 0)
    out_ref[...] = out[0:B, :].astype(out_ref.dtype)


def _tiles(w):
    rows, cols = w.shape
    return w.reshape(rows // 8, 8, cols // 128, 128).transpose(0, 2, 1, 3).reshape(-1, 8, 128)


@jax.jit
def pallas_gated_mix__mha_block_cached__moe_arch_mod__decode_kernel(
    A_x: jax.Array,
    A_k_cache: jax.Array,
    A_v_cache: jax.Array,
    A_wq: jax.Array,
    A_wo: jax.Array,
    B_x: jax.Array,
    B_w_r: jax.Array,
    B_w_gate: jax.Array,
    B_w_up: jax.Array,
    B_w_down: jax.Array,
    gate_w: jax.Array,
):
    del B_x
    dma_sem = pltpu.SemaphoreType.DMA
    out = pl.pallas_call(
        _kernel,
        out_shape=jax.ShapeDtypeStruct((B, D), BF16),
        in_specs=[pl.BlockSpec(memory_space=pl.ANY)] * 10,
        out_specs=pl.BlockSpec(memory_space=pltpu.VMEM),
        scratch_shapes=[
            pltpu.VMEM((SLOTS, B, CH, DH), BF16),
            pltpu.VMEM((D * H * DH // 1024, 8, 128), BF16),
            pltpu.VMEM((D * H * DH // 1024, 8, 128), BF16),
            pltpu.VMEM((D * F // 1024, 8, 128), BF16),
            pltpu.VMEM((D * F // 1024, 8, 128), BF16),
            pltpu.VMEM((D * F // 1024, 8, 128), BF16),
            pltpu.VMEM((B, D), BF16),
            pltpu.VMEM((D,), BF16),
            pltpu.VMEM((D,), BF16),
            pltpu.VMEM((M, D), F32),
            pltpu.VMEM((2, M, 128), F32),
            pltpu.VMEM((M, DH), BF16),
            pltpu.VMEM((M, 128), F32),
            pltpu.VMEM((M, 128), F32),
            pltpu.VMEM((M, DH), F32),
            pltpu.VMEM((H, M, DH), BF16),
            pltpu.VMEM((NC, M, CH), F32),
            pltpu.VMEM((B, F, 128), F32),
            pltpu.VMEM((M, D), F32),
            dma_sem((SLOTS,)),
            dma_sem((4,)),
            dma_sem((NR_FFN * NB,)),
            dma_sem((3,)),
        ],
        compiler_params=pltpu.CompilerParams(
            vmem_limit_bytes=96 * 1024 * 1024,
            disable_bounds_checks=True,
            disable_semaphore_checks=True),
    )(A_x.reshape(B, D), A_k_cache.reshape(-1, DH), A_v_cache.reshape(-1, DH),
      _tiles(A_wq), _tiles(A_wo), B_w_r, _tiles(B_w_gate), _tiles(B_w_up), _tiles(B_w_down),
      gate_w)
    return out.reshape(B, 1, D)
```

```python
import functools

import jax
import jax.experimental.pallas as pl
import jax.experimental.pallas.tpu as pltpu
import jax.numpy as jnp

B, D, H, SK, DH, F = 4, 1024, 32, 8192, 128, 3584

M = 8
BLK = 256
LEAD = 192
CUT = BLK - LEAD
NB = 8
G = 4
CH = G * BLK
NC = SK // CH
NS = 2 * NC
SLOTS = 2 * NS
AHEAD = 3
WD_AHEAD = 4

NR_FFN = D * F // (128 * NB * BLK)
NR_ATT = D * H * DH // (128 * NB * BLK)
EVERY = 8
T_ACT = (2 * NR_FFN + 1) * EVERY
T_OUT = (H - 1) * NS
assert (2 * NR_FFN + NR_ATT) * EVERY < T_OUT and T_ACT + F // 128 < T_OUT and AHEAD < NC

F32, BF16 = jnp.float32, jnp.bfloat16


def _plan(heavy, light):
    copies = []
    for queue, blocks, sizes, phase in ((1, range(NB - 1), heavy, 0.0), (0, [NB - 1], light, 0.5)):
        for i, s in enumerate(blocks):
            row = 0
            for rows in sizes:
                assert not row < CUT < row + rows
                copies.append(((i * BLK + row + phase * rows) / len(blocks), (s, row, rows, queue)))
                row += rows
            assert row == BLK
    return [copy for _, copy in sorted(copies)]


PLAN = _plan((CUT, LEAD), (32,) * 8)
FIRST_PLAN = _plan((32,) * 8, (16,) * 16)


def _kernel(x_hbm, k_hbm, v_hbm, wq_hbm, wo_hbm, wr_hbm, wg_hbm, wu_hbm, wd_hbm, gw_hbm,
            out_ref,
            ring, wq, wo, wg, wu, wd, x_in, wr, gw,
            xs, mix, qs, run_max, run_sum, run_pv, heads, scores, acts, a_acc,
            ring_sem, w_sem, wd_sem, small_sem):

    def wait_all(buf, sem):
        pltpu.make_async_copy(buf, buf, sem).wait()

    def tile_of(w, c, s, row):
        stride = w.shape[0] // NB
        tile = s * stride + (LEAD + row) // 8 + ((c & 1) * (stride // 2) + (c >> 1) * (BLK // 8))
        if s == NB - 1 and row >= CUT:
            tile = jnp.where(tile >= w.shape[0], tile - w.shape[0], tile)
        return tile

    def start_round(src, dst, sem_of, c, plan=PLAN):
        for s, row, rows, queue in plan:
            at = pl.ds(tile_of(dst, c, s, row), rows // 8)
            pltpu.make_async_copy(src.at[at], dst.at[at], sem_of(s)).start(priority=queue)

    def start_wd(c):
        start_round(wd_hbm, wd, lambda s: wd_sem.at[c * NB + s], c)

    def start_kv(src, h, c, slot):
        last = c == NC - 1
        next_slot = jnp.where(last, (slot + NS) % SLOTS, slot)
        in_range = jnp.logical_or(h < H - 1, jnp.logical_not(last))

        @pl.loop(0, B, step=NB // G)
        def _(b0):
            def start(s, row, rows, queue, slot):
                b, g = divmod(s, G)
                first = b * H * SK + g * (SK // G) + LEAD + row + ((b0 * H + h) * SK + c * BLK)
                pltpu.make_async_copy(src.at[pl.ds(pl.multiple_of(first, 16), rows)],
                                      ring.at[slot, b0 + b, pl.ds(g * BLK + row, rows)],
                                      ring_sem.at[slot]).start(priority=queue)

            for s, row, rows, queue in PLAN:
                if s % G == G - 1 and row >= CUT:
                    pl.when(in_range)(functools.partial(start, s, row, rows, queue, next_slot))
                else:
                    start(s, row, rows, queue, slot)

    def fold(a, op):
        return functools.reduce(op, [a[:, i:i + 128] for i in range(0, CH, 128)])

    def wide(a):
        return jnp.concatenate([a] * (D // 128), axis=1)

    def per_batch(fn):
        parts = [fn(b) for b in range(B)]
        row = jax.lax.broadcasted_iota(jnp.int32, parts[0].shape, 0)
        merged = jnp.zeros_like(parts[0])
        for b in range(B):
            merged = jnp.where(row == b, parts[b], merged)
        return merged

    def x_times(w, c):
        per_band = w.shape[0] // (D // 8)
        cols = jnp.concatenate([w[c + i * per_band] for i in range(D // 8)], axis=0)
        return jnp.dot(xs[...].astype(BF16), cols, preferred_element_type=F32)

    def project(h):
        n = D // 128
        rows = jnp.concatenate(
            [jnp.concatenate([wo[(h * (DH // 8) + i) * n + c] for i in range(DH // 8)], axis=0)
             for c in range(n)], axis=1)
        a_acc[...] += jnp.dot(heads[h], rows, preferred_element_type=F32)

    start_round(wq_hbm, wq, lambda s: w_sem.at[0], 0, FIRST_PLAN)
    pl.loop(1, NR_ATT)(functools.partial(start_round, wq_hbm, wq, lambda s: w_sem.at[0]))

    small = ((x_hbm, x_in), (wr_hbm, wr), (gw_hbm, gw))
    for i, (src, dst) in enumerate(small):
        pltpu.make_async_copy(src, dst, small_sem.at[i]).start()
    for src, slot in ((k_hbm, NC - 1), (v_hbm, NS - 1)):
        for b in range(B):
            pltpu.make_async_copy(src.at[pl.ds(b * H * SK, LEAD)],
                                  ring.at[slot, b, pl.ds(CH - LEAD, LEAD)],
                                  ring_sem.at[slot]).start(priority=b % 2)

    def consume(t):
        h, r, slot = t // NS, t % NS, t % SLOTS

        @pl.when(t == 0)
        def _():
            for i, (src, dst) in enumerate(small):
                pltpu.make_async_copy(src, dst, small_sem.at[i]).wait()
            xs[...] = jnp.zeros(xs.shape, F32)
            xs[0:B, :] = x_in[...].astype(F32)
            a_acc[...] = jnp.zeros(a_acc.shape, F32)
            wait_all(wq, w_sem.at[0])

        @pl.when(r == 0)
        def _():
            qs[...] = x_times(wq, h).astype(BF16)
            run_max[...] = jnp.full(run_max.shape, -jnp.inf, F32)
            run_sum[...] = jnp.zeros(run_sum.shape, F32)
            run_pv[...] = jnp.zeros(run_pv.shape, F32)

        @pl.when(r < NC)
        def _():
            wait_all(ring.at[slot], ring_sem.at[slot])
            q = qs[...]
            s = per_batch(lambda b: jax.lax.dot_general(
                q, ring[slot, b], (((1,), (1,)), ((), ())),
                preferred_element_type=F32)) * (DH ** -0.5)
            scores[r] = s
            run_max[...] = jnp.maximum(run_max[...], fold(s, jnp.maximum))

        @pl.when(r >= NC)
        def _():
            p = jnp.exp(scores[r - NC] - jnp.max(run_max[...], axis=-1, keepdims=True))
            run_sum[...] += fold(p, jnp.add)
            p16 = p.astype(BF16)
            wait_all(ring.at[slot], ring_sem.at[slot])
            run_pv[...] += per_batch(
                lambda b: jnp.dot(p16, ring[slot, b], preferred_element_type=F32))

    def request(t):
        h, r, slot = t // NS, t % NS, t % SLOTS
        pl.when(jnp.logical_and(h < H, r < NC))(functools.partial(start_kv, k_hbm, h, r, slot))
        pl.when(r >= NC)(functools.partial(start_kv, v_hbm, h, r - NC, slot))

        @pl.when(h == H)
        def _():
            pl.loop(jnp.minimum(2 * r, WD_AHEAD), jnp.minimum(2 * r + 2, WD_AHEAD))(start_wd)

    def side_jobs(t):
        h, r = t // NS, t % NS

        @pl.when(t % EVERY == 2)
        def _():
            c = t // EVERY
            for i, (src, dst, rounds) in enumerate(
                    ((wg_hbm, wg, NR_FFN), (wu_hbm, wu, NR_FFN), (wo_hbm, wo, NR_ATT)), 1):
                pl.when(jnp.logical_and(c >= 0, c < rounds))(
                    functools.partial(start_round, src, dst, lambda s: w_sem.at[i], c))
                c = c - rounds

        @pl.when(r == NS - 1)
        def _():
            denom = jnp.sum(run_sum[...], axis=-1, keepdims=True)
            heads[h] = (run_pv[...] / denom).astype(BF16)

        @pl.when(t == T_ACT - 1)
        def _():
            gate, router = [
                jax.nn.sigmoid(jnp.sum(xs[...] * w[...].astype(F32).reshape(1, D),
                                       axis=-1, keepdims=True)) for w in (gw, wr)]
            mix[0] = jnp.broadcast_to(gate, (M, 128))
            mix[1] = jnp.broadcast_to((1.0 - gate) * router, (M, 128))
            wait_all(wg, w_sem.at[1])
            wait_all(wu, w_sem.at[2])

        @pl.when(jnp.logical_and(t >= T_ACT, t < T_ACT + F // 128))
        def _():
            c = t - T_ACT
            g = x_times(wg, c)
            act = (g * jax.nn.sigmoid(g)) * x_times(wu, c) * mix[1]
            for b in range(B):
                acts[b, pl.ds(pl.multiple_of(c * 128, 128), 128), :] = (
                    jnp.broadcast_to(act[b:b + 1, :], (128, 128)).T)

        @pl.when(t == T_OUT)
        def _():
            wait_all(wo, w_sem.at[3])

        @pl.when(t >= T_OUT)
        def _():
            last = r == NS - 1
            lo = jnp.where(last, H - 1, jnp.minimum(r * 3, H - 1))
            hi = jnp.where(last, H, jnp.minimum((r + 1) * 3, H - 1))
            pl.loop(lo, hi)(project)

    @pl.loop(-AHEAD, H * NS)
    def _(t):
        pl.when(t >= 0)(functools.partial(consume, t))
        request(t + AHEAD)
        pl.when(t >= 0)(functools.partial(side_jobs, t))

    x, gate = xs[...], wide(mix[0])
    a_acc[...] = gate * a_acc[...] + (1.0 - gate) * (x + x * 0.0)

    def down(c, sums):
        pl.when(c + WD_AHEAD < NR_FFN)(functools.partial(start_wd, c + WD_AHEAD))
        for s in (NB - 1, *range(NB - 1)):
            for row, rows in ((0, CUT), (CUT, LEAD)) if s == NB - 1 else ((0, BLK),):
                wait_all(wd.at[pl.ds(tile_of(wd, c, s, row), rows // 8)], wd_sem.at[c * NB + s])
            for row in range(0, BLK, 8 * D // 128):
                tile = pl.multiple_of(tile_of(wd, c, s, row), 8)
                w = jnp.concatenate([wd[tile + k].astype(F32) for k in range(D // 128)], axis=1)
                sums = [sums[b] + wide(acts[b, pl.ds(tile, 8), :]) * w for b in range(B)]
        return sums

    sums = jax.lax.fori_loop(0, NR_FFN, down, [jnp.zeros((8, D), F32)] * B)

    def merge(u, v, k):
        low = (jax.lax.broadcasted_iota(jnp.int32, u.shape, 0) & k) == 0
        return jnp.where(low, u, v) + pltpu.roll(jnp.where(low, v, u), 8 - k, 0)

    y = merge(merge(sums[0], sums[1], 1), merge(sums[2], sums[3], 1), 2)
    out = a_acc[...] + y + pltpu.roll(y, 4, 0)
    out_ref[...] = out[0:B, :].astype(out_ref.dtype)


def _tiles(w):
    rows, cols = w.shape
    return w.reshape(rows // 8, 8, cols // 128, 128).transpose(0, 2, 1, 3).reshape(-1, 8, 128)


@jax.jit
def pallas_gated_mix__mha_block_cached__moe_arch_mod__decode_kernel(
    A_x: jax.Array,
    A_k_cache: jax.Array,
    A_v_cache: jax.Array,
    A_wq: jax.Array,
    A_wo: jax.Array,
    B_x: jax.Array,
    B_w_r: jax.Array,
    B_w_gate: jax.Array,
    B_w_up: jax.Array,
    B_w_down: jax.Array,
    gate_w: jax.Array,
):
    del B_x
    dma_sem = pltpu.SemaphoreType.DMA
    out = pl.pallas_call(
        _kernel,
        out_shape=jax.ShapeDtypeStruct((B, D), BF16),
        in_specs=[pl.BlockSpec(memory_space=pl.ANY)] * 10,
        out_specs=pl.BlockSpec(memory_space=pltpu.VMEM),
        scratch_shapes=[
            pltpu.VMEM((SLOTS, B, CH, DH), BF16),
            pltpu.VMEM((D * H * DH // 1024, 8, 128), BF16),
            pltpu.VMEM((D * H * DH // 1024, 8, 128), BF16),
            pltpu.VMEM((D * F // 1024, 8, 128), BF16),
            pltpu.VMEM((D * F // 1024, 8, 128), BF16),
            pltpu.VMEM((D * F // 1024, 8, 128), BF16),
            pltpu.VMEM((B, D), BF16),
            pltpu.VMEM((D,), BF16),
            pltpu.VMEM((D,), BF16),
            pltpu.VMEM((M, D), F32),
            pltpu.VMEM((2, M, 128), F32),
            pltpu.VMEM((M, DH), BF16),
            pltpu.VMEM((M, 128), F32),
            pltpu.VMEM((M, 128), F32),
            pltpu.VMEM((M, DH), F32),
            pltpu.VMEM((H, M, DH), BF16),
            pltpu.VMEM((NC, M, CH), F32),
            pltpu.VMEM((B, F, 128), F32),
            pltpu.VMEM((M, D), F32),
            dma_sem((SLOTS,)),
            dma_sem((4,)),
            dma_sem((NR_FFN * NB,)),
            dma_sem((3,)),
        ],
        compiler_params=pltpu.CompilerParams(
            vmem_limit_bytes=96 * 1024 * 1024,
            disable_bounds_checks=True,
            disable_semaphore_checks=True),
    )(A_x.reshape(B, D), A_k_cache.reshape(-1, DH), A_v_cache.reshape(-1, DH),
      _tiles(A_wq), _tiles(A_wo), B_w_r, _tiles(B_w_gate), _tiles(B_w_up), _tiles(B_w_down),
      gate_w)
    return out.reshape(B, 1, D)
```

```python
import functools

import jax
import jax.experimental.pallas as pl
import jax.experimental.pallas.tpu as pltpu
import jax.numpy as jnp

B, D, H, SK, DH, F = 4, 1024, 32, 8192, 128, 3584

M = 8
BLK = 256
LEAD = 192
CUT = BLK - LEAD

G = 4
CH = G * BLK
NC = SK // CH
STEPS = H * NC
SLOTS = 2 * NC
AHEAD = 3
KV_COPIES = ((0, CUT, 1), (CUT, 32, 0), (CUT + 32, LEAD - 32, 1))
LAG = 13

NB = 8
WD_AHEAD = 5
assert CH == D and NC == D // 128 and AHEAD < NC and F // 128 <= STEPS - AHEAD

F32, BF16 = jnp.float32, jnp.bfloat16


def _plan(heavy, light):
    copies = []
    for queue, blocks, sizes, phase in ((1, range(NB - 1), heavy, 0.0), (0, [NB - 1], light, 0.5)):
        for i, s in enumerate(blocks):
            row = 0
            for rows in sizes:
                assert not row < CUT < row + rows
                copies.append(((i * BLK + row + phase * rows) / len(blocks), (s, row, rows, queue)))
                row += rows
            assert row == BLK
    return [copy for _, copy in sorted(copies)]


PLAN = _plan((CUT, LEAD), (32,) * 8)
FIRST_PLAN = _plan((32,) * 8, (16,) * 16)


def _kernel(x_hbm, k_hbm, v_hbm, wq_hbm, wo_hbm, wr_hbm, wg_hbm, wu_hbm, wd_hbm, gw_hbm,
            out_ref,
            ring, wq, wo, wg, wu, wd, x_in, wr, gw,
            xs, qs, run_max, run_sum, run_pv, head, a_acc, acts,
            ring_sem, w_sem, wd_sem, small_sem):

    def wait_all(buf, sem):
        pltpu.make_async_copy(buf, buf, sem).wait()

    def rounds(w):
        return w.shape[0] * 8 // (NB * BLK)

    def tile_of(w, c, s, row):
        stride = w.shape[0] // NB
        tile = s * stride + (LEAD + row) // 8 + ((c & 1) * (stride // 2) + (c >> 1) * (BLK // 8))
        if s == NB - 1 and row >= CUT:
            tile = jnp.where(tile >= w.shape[0], tile - w.shape[0], tile)
        return tile

    def start_round(src, dst, sem_of, c, plan=PLAN):
        for s, row, rows, queue in plan:
            at = pl.ds(tile_of(dst, c, s, row), rows // 8)
            pltpu.make_async_copy(src.at[at], dst.at[at], sem_of(s)).start(priority=queue)

    def start_wd(c):
        start_round(wd_hbm, wd, lambda s: wd_sem.at[c * NB + s], c)

    def start_kv(t, block, row, rows, queue):
        kv, b, g = block // (B * G), block // G % B, block % G
        c, slot = t % NC, t % SLOTS

        def start(slot):
            first = b * H * SK + g * (SK // G) + LEAD + row + (t // NC * SK + c * BLK)
            pltpu.make_async_copy((k_hbm, v_hbm)[kv].at[pl.ds(pl.multiple_of(first, 16), rows)],
                                  ring.at[slot, kv, b, pl.ds(g * BLK + row, rows)],
                                  ring_sem.at[slot]).start(priority=queue)

        if g == G - 1 and row >= CUT:
            pl.when(t < STEPS - 1)(functools.partial(
                start, jnp.where(c == NC - 1, (t + NC) % SLOTS, slot)))
        else:
            start(slot)

    def request(t, block, this=True, previous=True):
        for row, rows, queue in KV_COPIES:
            due = block if queue else block - LAG
            if due < 0:
                pl.when(previous)(functools.partial(
                    start_kv, t - 1, due + 2 * B * G, row, rows, queue))
            elif this:
                start_kv(t, due, row, rows, queue)

    def fold(a, op):
        return functools.reduce(op, [a[:, i:i + 128] for i in range(0, CH, 128)])

    def wide(a):
        return jnp.concatenate([a] * (D // 128), axis=1)

    def per_batch(fn):
        parts = [fn(b) for b in range(B)]
        row = jax.lax.broadcasted_iota(jnp.int32, parts[0].shape, 0)
        merged = jnp.zeros_like(parts[0])
        for b in range(B):
            merged = jnp.where(row == b, parts[b], merged)
        return merged

    def x_times(w, c):
        per_band = w.shape[0] // (D // 8)
        cols = jnp.concatenate([w[c + i * per_band] for i in range(D // 8)], axis=0)
        return jnp.dot(xs[...].astype(BF16), cols, preferred_element_type=F32)

    def project(h, c):
        w = jnp.concatenate(
            [wo[(h * (DH // 8) + i) * (D // 128) + c] for i in range(DH // 8)], axis=0)
        return jnp.dot(head[...], w, preferred_element_type=F32)

    def attend(t, after_block):
        h, c, slot = t // NC, t % NC, t % SLOTS

        def blocks(kv, b, fn):
            out = []
            for g in range(G):
                out.append(fn(g, ring[slot, kv, b, g * BLK:(g + 1) * BLK, :]))
                after_block((kv * B + b) * G + g)
            return out

        @pl.when(c == 0)
        def _():
            qs[...] = x_times(wq, h).astype(BF16)
            run_max[...] = jnp.full(run_max.shape, -jnp.inf, F32)
            run_sum[...] = jnp.zeros(run_sum.shape, F32)
            run_pv[...] = jnp.zeros(run_pv.shape, F32)

        wait_all(ring.at[slot], ring_sem.at[slot])
        q = qs[...]
        s = per_batch(lambda b: jnp.concatenate(blocks(0, b, lambda g, k: jax.lax.dot_general(
            q, k, (((1,), (1,)), ((), ())), preferred_element_type=F32)), axis=1)) * (DH ** -0.5)
        a_acc[c] = jnp.where(h > 0, a_acc[c] + project(jnp.maximum(h - 1, 0), c), 0.0)

        old_max = run_max[...]
        new_max = jnp.maximum(old_max, jnp.max(fold(s, jnp.maximum), axis=-1, keepdims=True))
        keep = jnp.exp(old_max - new_max)
        p = jnp.exp(s - wide(new_max))
        p16 = p.astype(BF16)
        run_max[...] = new_max
        run_sum[...] = keep * run_sum[...] + fold(p, jnp.add)
        run_pv[...] = keep * run_pv[...] + per_batch(
            lambda b: functools.reduce(jnp.add, blocks(1, b, lambda g, v: jnp.dot(
                p16[:, g * BLK:(g + 1) * BLK], v, preferred_element_type=F32))))

        @pl.when(c == NC - 1)
        def _():
            denom = jnp.sum(run_sum[...], axis=-1, keepdims=True)
            head[...] = (run_pv[...] / denom).astype(BF16)

    first = ((wq_hbm, wq), (wg_hbm, wg), (wu_hbm, wu), (wo_hbm, wo))
    start_round(wq_hbm, wq, lambda s: w_sem.at[0], 0, FIRST_PLAN)
    small = [pltpu.make_async_copy(src, dst, small_sem.at[i])
             for i, (src, dst) in enumerate(((x_hbm, x_in), (wr_hbm, wr), (gw_hbm, gw)))]
    for copy in small:
        copy.start()
    for i, (src, dst) in enumerate(first):
        pl.loop(0 if i else 1, rounds(dst))(
            functools.partial(start_round, src, dst, lambda s: w_sem.at[i]))
    for kv, src in enumerate((k_hbm, v_hbm)):
        for b in range(B):
            pltpu.make_async_copy(src.at[pl.ds(b * H * SK, LEAD)],
                                  ring.at[NC - 1, kv, b, pl.ds(CH - LEAD, LEAD)],
                                  ring_sem.at[NC - 1]).start(priority=b % 2)

    for copy in small:
        copy.wait()
    for ref in (xs, head, a_acc):
        ref[...] = jnp.zeros(ref.shape, ref.dtype)
    xs[0:B, :] = x_in[...].astype(F32)
    gate, router = [
        jax.nn.sigmoid(jnp.sum(xs[...] * w[...].astype(F32).reshape(1, D), axis=-1, keepdims=True))
        for w in (gw, wr)]

    @pl.loop(0, AHEAD)
    def _(t):
        for block in range(2 * B * G):
            request(t, block, previous=t > 0)

    for i, (_, dst) in enumerate(first):
        wait_all(dst, w_sem.at[i])

    @pl.loop(0, STEPS - AHEAD)
    def _(t):
        attend(t, functools.partial(request, t + AHEAD))

        @pl.when(t < F // 128)
        def _():
            g = x_times(wg, t)
            act = (g * jax.nn.sigmoid(g)) * x_times(wu, t) * ((1.0 - gate) * router)
            for b in range(B):
                acts[b, pl.ds(pl.multiple_of(t * 128, 128), 128), :] = (
                    jnp.broadcast_to(act[b:b + 1, :], (128, 128)).T)

    for block in range(LAG):
        request(STEPS, block, this=False)

    @pl.loop(0, AHEAD)
    def _(i):
        pl.loop(i * WD_AHEAD // AHEAD, (i + 1) * WD_AHEAD // AHEAD)(start_wd)
        attend(STEPS - AHEAD + i, lambda block: None)

    a = jnp.concatenate([a_acc[c] + project(H - 1, c) for c in range(D // 128)], axis=1)
    x = xs[...]
    rest = gate * a + (1.0 - gate) * (x + x * 0.0)

    def down(c, sums):
        pl.when(c + WD_AHEAD < rounds(wd))(functools.partial(start_wd, c + WD_AHEAD))
        for s in (NB - 1, *range(NB - 1)):
            for row, rows in ((0, CUT), (CUT, LEAD)) if s == NB - 1 else ((0, BLK),):
                wait_all(wd.at[pl.ds(tile_of(wd, c, s, row), rows // 8)], wd_sem.at[c * NB + s])
            for row in range(0, BLK, 8 * D // 128):
                tile = pl.multiple_of(tile_of(wd, c, s, row), 8)
                w = jnp.concatenate([wd[tile + k].astype(F32) for k in range(D // 128)], axis=1)
                sums = [sums[b] + wide(acts[b, pl.ds(tile, 8), :]) * w for b in range(B)]
        return sums

    sums = jax.lax.fori_loop(0, rounds(wd), down, [jnp.zeros((8, D), F32)] * B)

    def merge(u, v, k):
        low = (jax.lax.broadcasted_iota(jnp.int32, u.shape, 0) & k) == 0
        return jnp.where(low, u, v) + pltpu.roll(jnp.where(low, v, u), 8 - k, 0)

    y = merge(merge(sums[0], sums[1], 1), merge(sums[2], sums[3], 1), 2)
    out = rest + y + pltpu.roll(y, 4, 0)
    out_ref[...] = out[0:B, :].astype(out_ref.dtype)


def _tiles(w):
    rows, cols = w.shape
    return w.reshape(rows // 8, 8, cols // 128, 128).transpose(0, 2, 1, 3).reshape(-1, 8, 128)


@jax.jit
def pallas_gated_mix__mha_block_cached__moe_arch_mod__decode_kernel(
    A_x: jax.Array,
    A_k_cache: jax.Array,
    A_v_cache: jax.Array,
    A_wq: jax.Array,
    A_wo: jax.Array,
    B_x: jax.Array,
    B_w_r: jax.Array,
    B_w_gate: jax.Array,
    B_w_up: jax.Array,
    B_w_down: jax.Array,
    gate_w: jax.Array,
):
    del B_x
    dma_sem = pltpu.SemaphoreType.DMA
    out = pl.pallas_call(
        _kernel,
        out_shape=jax.ShapeDtypeStruct((B, D), BF16),
        in_specs=[pl.BlockSpec(memory_space=pl.ANY)] * 10,
        out_specs=pl.BlockSpec(memory_space=pltpu.VMEM),
        scratch_shapes=[
            pltpu.VMEM((SLOTS, 2, B, CH, DH), BF16),
            pltpu.VMEM((D * H * DH // 1024, 8, 128), BF16),
            pltpu.VMEM((D * H * DH // 1024, 8, 128), BF16),
            pltpu.VMEM((D * F // 1024, 8, 128), BF16),
            pltpu.VMEM((D * F // 1024, 8, 128), BF16),
            pltpu.VMEM((D * F // 1024, 8, 128), BF16),
            pltpu.VMEM((B, D), BF16),
            pltpu.VMEM((D,), BF16),
            pltpu.VMEM((D,), BF16),
            pltpu.VMEM((M, D), F32),
            pltpu.VMEM((M, DH), BF16),
            pltpu.VMEM((M, 128), F32),
            pltpu.VMEM((M, 128), F32),
            pltpu.VMEM((M, DH), F32),
            pltpu.VMEM((M, DH), BF16),
            pltpu.VMEM((D // 128, M, 128), F32),
            pltpu.VMEM((B, F, 128), F32),
            dma_sem((SLOTS,)),
            dma_sem((4,)),
            dma_sem((F * D // (128 * BLK),)),
            dma_sem((3,)),
        ],
        compiler_params=pltpu.CompilerParams(
            vmem_limit_bytes=96 * 1024 * 1024,
            disable_bounds_checks=True,
            disable_semaphore_checks=True),
    )(A_x.reshape(B, D), A_k_cache.reshape(-1, DH), A_v_cache.reshape(-1, DH),
      _tiles(A_wq), _tiles(A_wo), B_w_r, _tiles(B_w_gate), _tiles(B_w_up), _tiles(B_w_down),
      gate_w)
    return out.reshape(B, 1, D)
```
